```python
import jax
import jax.numpy as jnp

def _softmax(x, axis=-1):
    return jax.nn.softmax(x, axis=axis)
def _gelu(x):
    return jax.nn.gelu(x, approximate=True)
def _silu(x):
    return jax.nn.silu(x)
def _sigmoid(x):
    return jax.nn.sigmoid(x)
def _layernorm(x, axis=-1, eps=1e-5):
    m = jnp.mean(x, axis=axis, keepdims=True)
    v = jnp.var(x, axis=axis, keepdims=True)
    return (x - m) / jnp.sqrt(v + eps)
def _scatter_add(tgt, idx, src, axis=0):
    return tgt.at[idx].add(src)
def _segment_sum(src, seg, n):
    return jax.ops.segment_sum(src, seg, n)
class _Rng:
    def __init__(self, key):
        self._k = key
    def _next(self):
        self._k, sub = jax.random.split(self._k)
        return sub
    def normal(self, shape):
        return jax.random.normal(self._next(), shape, dtype=jnp.bfloat16)
    def randint(self, lo, hi, shape):
        return jax.random.randint(self._next(), shape, lo, hi, dtype=jnp.int32)
    def uniform(self, shape, lo=0.0, hi=1.0):
        return jax.random.uniform(self._next(), shape, jnp.bfloat16, lo, hi)
    def permutation(self, n):
        return jax.random.permutation(self._next(), n)


kernel_name = 'interleave_layers__sliding_local_dilated__dense_activation_gelu__prompt'

def setup_inputs():
    _rng = _Rng(jax.random.key(int.from_bytes(__import__("os").urandom(4), "little")))
    _w = (lambda a: (lambda t: t.astype(jnp.bfloat16) if jnp.issubdtype(t.dtype, jnp.floating) else t)(jnp.asarray(a)))
    def _A_setup():
        B, S, D = 1, 2048, 1024
        return {
            "x": _w((lambda *s: _rng.normal(s) * 0.05)(B, S, D)),
            "wqkv": _w((lambda *s: _rng.normal(s) * 0.05)(D, 3 * D)),
            "wo": _w((lambda *s: _rng.normal(s) * 0.05)(D, D)),
        }
    _A_in = _A_setup()

    def _B_setup():
        B, S, D, F = 1, 2048, 1024, 3584
        return {
            "x": _w((lambda *s: _rng.normal(s) * 0.05)(B, S, D)),
            "w1": _w((lambda *s: _rng.normal(s) * 0.05)(D, F) * (D ** -0.5)),
            "b1": _w((lambda *s: _rng.normal(s) * 0.05)(F) * 0.01),
            "w2": _w((lambda *s: _rng.normal(s) * 0.05)(F, D) * (F ** -0.5)),
            "b2": _w((lambda *s: _rng.normal(s) * 0.05)(D) * 0.01),
        }
    _B_in = _B_setup()

    return {
        "A_x": _A_in["x"],
        "A_wqkv": _A_in["wqkv"],
        "A_wo": _A_in["wo"],
        "B_x": _B_in["x"],
        "B_w1": _B_in["w1"],
        "B_b1": _B_in["b1"],
        "B_w2": _B_in["w2"],
        "B_b2": _B_in["b2"],
    }

def reference(A_x, A_wqkv, A_wo, B_x, B_w1, B_b1, B_w2, B_b2):
    def _A_ref(x, wqkv, wo):
        B, S, D = x.shape
        H = 32; Dh = D // H
        W, dil = 8, 2
        qkv = (lambda x, *d: x.transpose(*d))((x @ wqkv).reshape(B, S, 3, H, Dh), 2, 0, 3, 1, 4)
        q, k, v = qkv[0], qkv[1], qkv[2]
        scale = Dh ** -0.5
        pos = jnp.arange(S)
        off = jnp.arange(W) * dil
        idx = pos[:, None] - off[None, :]
        mask = idx >= 0
        idx_c = jnp.where(mask, idx, 0).reshape(-1)
        kg = k[:, :, idx_c, :].reshape(B, H, S, W, Dh)
        vg = v[:, :, idx_c, :].reshape(B, H, S, W, Dh)
        logits = jnp.einsum("bhsd,bhswd->bhsw", q, kg) * scale
        logits = jnp.where(mask[None, None, :, :], logits, -1e9)
        attn = _softmax(logits, axis=-1)
        o = jnp.einsum("bhsw,bhswd->bhsd", attn, vg)
        return (lambda x, *d: x.transpose(*d))(o, 0, 2, 1, 3).reshape(B, S, D) @ wo

    def _B_ref(x, w1, b1, w2, b2):
        h = jnp.einsum("bsd,df->bsf", x, w1) + b1
        h = _gelu(h)
        return jnp.einsum("bsf,fd->bsd", h, w2) + b2

    x = A_x
    x = x + _A_ref(_layernorm(x, axis=-1), A_wqkv, A_wo)
    x = x + _B_ref(_layernorm(x, axis=-1), B_w1, B_b1, B_w2, B_b2)
    x = x + _A_ref(_layernorm(x, axis=-1), A_wqkv, A_wo)
    x = x + _B_ref(_layernorm(x, axis=-1), B_w1, B_b1, B_w2, B_b2)
    return x
```

```python
import functools
import jax
import jax.numpy as jnp
from jax import lax
import jax.experimental.pallas as pl
import jax.experimental.pallas.tpu as pltpu

T = 256
FC = 512
H = 32; DH = 32; W = 8; DIL = 2; HALO = 16
RB = 16
WSPLIT = 4
PW = 1024; SB = 32; LB = 16
PIN = 1
NPRE = 2; A0 = 7; L0 = 4; F0 = 1
CH = 1
AD = 1; LD = 1; LB2 = 32; LD2 = 1
SQ = 0; SP = 0
F32 = jnp.float32; BF16 = jnp.bfloat16; U32 = jnp.uint32


def _ln(x):
    m = jnp.mean(x, axis=-1, keepdims=True)
    xc = x - m
    v = jnp.mean(xc * xc, axis=-1, keepdims=True)
    return xc * lax.rsqrt(v + 1e-5)


def _gelu(x):
    c = 0.7978845608028654
    return 0.5 * x * (1.0 + jnp.tanh(c * (x + 0.044715 * (x * x * x))))


def _dot(a, b):
    return jnp.dot(a, b, preferred_element_type=F32)


def kernel(x_hbm, wqkv_hbm, wo_hbm, w1_hbm, b1_ref, w2_hbm, b2_ref, out_hbm,
           wqkv, wo, w1, w2, xin, xs, obuf, qkv, xn1, osc, acc_s, xn2_s, tmp,
           sem_x, sem_w, sem_f, sem_o):
    S, D = xin.shape
    G = D // 128
    NT = S // T
    NC = w1.shape[0]
    NU = 2 * NT

    def x_copy(t):
        return pltpu.make_async_copy(x_hbm.at[pl.ds(t * T, T), :], xin.at[pl.ds(t * T, T), :], sem_x.at[t])

    def wqkv_copy(j):
        return pltpu.make_async_copy(wqkv_hbm.at[:, pl.ds(j * D, D)], wqkv.at[j], sem_w.at[j])

    def wo_copy():
        return pltpu.make_async_copy(wo_hbm, wo, sem_w.at[3])

    def w1_copy(c):
        return pltpu.make_async_copy(w1_hbm.at[:, pl.ds(c * FC, FC)], w1.at[c], sem_f.at[2 * c])

    def w2_copy(c):
        return pltpu.make_async_copy(w2_hbm.at[pl.ds(c * FC, FC), :], w2.at[c], sem_f.at[2 * c + 1])

    def out_copy(t):
        return pltpu.make_async_copy(obuf.at[pl.ds(t * T, T), :], out_hbm.at[pl.ds(t * T, T), :], sem_o.at[t])

    x_copy(0).start()
    wqkv_copy(0).start()
    wqkv_copy(1).start()
    wqkv_copy(2).start()
    x_copy(1).start()
    wo_copy().start()
    x_copy(2).start()
    for c in range(NC):
        w1_copy(c).start()
        w2_copy(c).start()
    for t in range(3, NT):
        x_copy(t).start()

    def lanes(n):
        return lax.broadcasted_iota(jnp.int32, (n, 128), 1)

    def fold(t):
        parts = [t[a:a + 8, b:b + 128] for a in range(0, t.shape[0], 8) for b in range(0, t.shape[1], 128)]
        return functools.reduce(jnp.bitwise_or, parts)

    def pin(ref, toks, never):
        toks = [t for t in toks if t is not None]
        if toks and PIN:
            tok = pltpu.bitcast(functools.reduce(jnp.bitwise_or, toks), BF16)
            ref[0:16, 0:128] = jnp.where(never, tok, ref[0:16, 0:128])

    def shuffle_store(j, src, r0, n):
        lane = lanes(n)
        v = [src[pl.ds(r0, n), g * 128:(g + 1) * 128] for g in range(G)]
        for k in range(3):
            m = (lane & (4 << k)) != 0
            v = [jnp.where(m, v[(g + (1 << k)) % G], v[g]) for g in range(G)]
        for gp in range(G):
            idx = (lane & 3) * 32 + (((lane >> 2) - gp) & 7) * 4 + (lane >> 5)
            v[gp] = jnp.take_along_axis(v[gp], idx, axis=1)
            qkv[j, gp, pl.ds(HALO + r0, n), :] = v[gp]
        return fold(pltpu.bitcast(functools.reduce(jnp.maximum, v), U32))

    def load_x(u, r0, n):
        r = pl.multiple_of((u % NT) * T + r0, n)
        return jnp.where(u < NT, xin[pl.ds(r, n), :].astype(F32), xs[pl.ds(r, n), :])

    scale = DH ** -0.5

    def gate(x, link):
        if link is not None and link['tok'] is not None:
            return jnp.where(link['never'], link['tok'], x)
        return x

    def chain_sum(terms, link, serial):
        if link is None:
            return functools.reduce(lambda a, b: a + b, terms)
        if not serial:
            acc = functools.reduce(lambda a, b: a + b, terms[1:], gate(terms[0], link))
            link['tok'] = acc
            return acc
        parts = []
        if link['tok'] is not None:
            link['tok'] = link['tok'][RB - 8:RB]
        for a in range(0, RB, 8):
            acc = functools.reduce(lambda x, y: x + y, [t[a:a + 8] for t in terms[1:]], gate(terms[0][a:a + 8], link))
            link['tok'] = acc
            parts.append(acc)
        link['tok'] = jnp.concatenate([acc] * (RB // 8), axis=0)
        return jnp.concatenate(parts, axis=0)

    def attn_qk(tile, rb, link):
        r0 = HALO + rb * RB
        lg = []
        for w in range(W):
            acc = chain_sum([qkv[0, g, pl.ds(r0, RB), :] * qkv[1, g, pl.ds(r0 - DIL * w, RB), :]
                             for g in range(G)], link, w % SQ == 0 if SQ else False)
            acc = acc + pltpu.roll(acc, 32, 1)
            acc = acc + pltpu.roll(acc, 64, 1)
            acc = acc * scale
            if rb * RB < DIL * w:
                pos = tile * T + rb * RB + lax.broadcasted_iota(jnp.int32, (RB, 128), 0)
                acc = jnp.where(pos >= DIL * w, acc, -1e9)
            lg.append(acc)
        m = functools.reduce(jnp.maximum, lg)
        e = [jnp.exp(a - m) for a in lg]
        s = functools.reduce(lambda a, b: a + b, e)
        inv = 1.0 / s
        return [a * inv for a in e]

    def attn_pv(rb, p, link):
        r0 = HALO + rb * RB
        lane = lanes(RB // 2)
        o = []
        for gp in range(G):
            acc = chain_sum([p[w] * qkv[2, gp, pl.ds(r0 - DIL * w, RB), :] for w in range(W)],
                            link, gp % SP == 0 if SP else False)
            pk = pltpu.bitcast(acc.astype(BF16), U32)
            idx = (lane & 3) * 32 + (((lane >> 2) + gp) & 7) * 4 + (lane >> 5)
            o.append(jnp.take_along_axis(pk, idx, axis=1))
        for k in range(3):
            m = (lane & (4 << k)) != 0
            o = [jnp.where(m, o[(g - (1 << k)) % G], o[g]) for g in range(G)]
        osc[pl.ds(rb * RB // 2, RB // 2), :] = jnp.concatenate(o, axis=1)
        return pltpu.bitcast(o[0], F32)

    def attention(tile, never):
        link = None if never is None else {'never': never, 'tok': None}
        nb = T // RB
        ps = {}
        done = {}
        for i in range(nb + AD):
            if i < nb:
                ps[i] = attn_qk(tile, i, link)
            if i >= AD:
                j = i - AD
                if link is not None and j >= 2:
                    link['tok'] = jnp.maximum(link['tok'], jnp.concatenate([done[j - 2]] * (RB // 8), axis=0))
                done[j] = attn_pv(j, ps.pop(j), link)

    def ln_chain(load, dst, lb, dist, never):
        outs = []
        for t, r0 in enumerate(range(0, T, lb)):
            x = load(r0, lb)
            if t >= dist:
                x0 = jnp.where(never, outs[t - dist], x[0:8, 0:128])
                x = jnp.concatenate([jnp.concatenate([x0, x[0:8, 128:]], axis=1), x[8:]], axis=0)
            y = _ln(x).astype(BF16)
            dst[pl.ds(r0, lb), :] = y
            outs.append(pltpu.bitcast(fold(pltpu.bitcast(y, U32)), F32))
        return pltpu.bitcast(outs[-1], U32)

    def o_val():
        return pltpu.bitcast(osc[...], BF16)

    def interleave(mm, vp, ref, never, first, last):
        n = len(vp)
        dl = [first + (t * (last + 1 - first)) // n for t in range(n)]
        for i in range(len(mm) + 1):
            toks = [t() for t, d in zip(vp, dl) if d == i]
            if i < len(mm):
                pin(ref, toks, never)
                mm[i]()

    NP = D // PW

    def proj_piece(j, p):
        def f():
            tmp[j, :, p * PW:(p + 1) * PW] = _dot(xn1[...], wqkv[j, :, p * PW:(p + 1) * PW])
        return f

    def ffn_chunk(xn2, c):
        h = _dot(xn2, w1[c])
        h = _gelu(h + b1_ref[c].astype(F32)).astype(BF16)
        return _dot(h, w2[c])

    qkv[:, :, 0:HALO, :] = jnp.zeros((3, G, HALO, 128), F32)
    x_copy(0).wait()
    xn1[...] = _ln(xin[0:T, :].astype(F32)).astype(BF16)

    def pro_body(j, carry):
        wqkv_copy(j).wait()
        acc_s[...] = _dot(xn1[...], wqkv[j])
        for r0 in range(0, T, SB):
            shuffle_store(j, acc_s, r0, SB)
        return carry
    lax.fori_loop(0, 3, pro_body, 0)
    x_copy(1).wait()
    xn1[...] = _ln(xin[T:2 * T, :].astype(F32)).astype(BF16)
    wo_copy().wait()

    def step(u, carry):
        tile = u % NT
        r = pl.multiple_of(tile * T, T)

        @pl.when(u + 2 < NT)
        def _():
            x_copy(u + 2).wait()

        never = u < 0
        pieces = [proj_piece(j, p) for j in range(3) for p in range(NP)]
        for f in pieces[:NPRE]:
            f()
        attention(tile, never)
        acc_s[...] = load_x(u, 0, T) + _dot(o_val(), wo[...])
        for f in pieces[NPRE:]:
            f()
        ln_chain(lambda r0, n: acc_s[pl.ds(r0, n), :], xn2_s, LB2, LD2, never)

        keep = (u + 1) % NT != 0
        u2 = jnp.minimum(u + 2, NU - 1)

        def halo(j):
            qkv[j, :, 0:HALO, :] = jnp.where(keep, qkv[j, :, T:T + HALO, :], 0.0)

        st = {'acc': None}

        def chunk(c):
            def f():
                if c in (0, WSPLIT):
                    @pl.when(u == 0)
                    def _():
                        for cc in (range(0, WSPLIT) if c == 0 else range(WSPLIT, NC)):
                            w1_copy(cc).wait()
                            w2_copy(cc).wait()
                if c == 0:
                    st['acc'] = acc_s[...] + b2_ref[...].astype(F32)
                st['acc'] = st['acc'] + ffn_chunk(xn2_s[...], c)
            return f
        tasks = ([functools.partial(halo, j) for j in (1, 2)]
                 + [functools.partial(shuffle_store, j, tmp.at[j], r0, SB) for j in range(3) for r0 in range(0, T, SB)]
                 + [functools.partial(ln_chain, functools.partial(load_x, u2), xn1, LB, LD, never)])
        interleave([chunk(c) for c in range(NC)], tasks, xn2_s, never, F0, NC - 1)
        xs[pl.ds(r, T), :] = st['acc']
        obuf[pl.ds(r, T), :] = st['acc'].astype(BF16)

        @pl.when(u >= NT)
        def _():
            out_copy(tile).start()
        return carry
    lax.fori_loop(0, NU - 1, step, 0)

    attention(NT - 1, None)
    x1 = xs[S - T:S, :] + _dot(o_val(), wo[...])
    xn2_s[...] = _ln(x1).astype(BF16)
    acc_s[...] = x1 + b2_ref[...].astype(F32)

    def epi_body(c, carry):
        acc_s[...] += ffn_chunk(xn2_s[...], c)
        return carry
    lax.fori_loop(0, NC, epi_body, 0)
    obuf[S - T:S, :] = acc_s[...].astype(BF16)
    out_copy(NT - 1).start()
    for t in range(NT):
        out_copy(t).wait()


@jax.jit
def pallas_interleave_layers__sliding_local_dilated__dense_activation_gelu__prompt_kernel(
        A_x, A_wqkv, A_wo, B_x, B_w1, B_b1, B_w2, B_b2):
    B, S, D = A_x.shape
    F = B_w1.shape[1]
    G = D // 128
    NC = F // FC
    NT = S // T
    hbm = pl.BlockSpec(memory_space=pl.ANY)
    vmem = pl.BlockSpec(memory_space=pltpu.VMEM)
    out = pl.pallas_call(
        kernel,
        in_specs=[hbm, hbm, hbm, hbm, vmem, hbm, vmem],
        out_specs=hbm,
        out_shape=jax.ShapeDtypeStruct((S, D), A_x.dtype),
        scratch_shapes=[pltpu.VMEM((3, D, D), BF16),
                        pltpu.VMEM((D, D), BF16),
                        pltpu.VMEM((NC, D, FC), BF16),
                        pltpu.VMEM((NC, FC, D), BF16),
                        pltpu.VMEM((S, D), BF16),
                        pltpu.VMEM((S, D), F32),
                        pltpu.VMEM((S, D), BF16),
                        pltpu.VMEM((3, G, T + HALO, 128), F32),
                        pltpu.VMEM((T, D), BF16),
                        pltpu.VMEM((T // 2, D), U32),
                        pltpu.VMEM((T, D), F32),
                        pltpu.VMEM((T, D), BF16),
                        pltpu.VMEM((3, T, D), F32),
                        pltpu.SemaphoreType.DMA((NT,)),
                        pltpu.SemaphoreType.DMA((4,)),
                        pltpu.SemaphoreType.DMA((2 * NC,)),
                        pltpu.SemaphoreType.DMA((NT,))],
        compiler_params=pltpu.CompilerParams(vmem_limit_bytes=100 * 1024 * 1024),
    )(A_x.reshape(S, D), A_wqkv, A_wo, B_w1, B_b1.reshape(NC, 1, FC), B_w2, B_b2.reshape(1, D))
    return out.reshape(B, S, D)
```

```python
import functools
import jax
import jax.numpy as jnp
from jax import lax
import jax.experimental.pallas as pl
import jax.experimental.pallas.tpu as pltpu

T = 256
FC = 512
H = 32; DH = 32; W = 8; DIL = 2; HALO = 16
RB = 16
WSPLIT = 4
PW = 1024; SB = 32; LB = 16
PIN = 1
NPRE = 2; A0 = 7; L0 = 4; F0 = 1
CH = 1
AD = 1; LD = 1; LB2 = 32; LD2 = 1
SQ = 0; SP = 0
EPI = 1; NIT = 0
DQ = 9
EP2 = 1; XW = 1
F32 = jnp.float32; BF16 = jnp.bfloat16; U32 = jnp.uint32


def _ln(x):
    m = jnp.mean(x, axis=-1, keepdims=True)
    xc = x - m
    v = jnp.mean(xc * xc, axis=-1, keepdims=True)
    return xc * lax.rsqrt(v + 1e-5)


def _gelu(x):
    c = 0.7978845608028654
    return 0.5 * x * (1.0 + jnp.tanh(c * (x + 0.044715 * (x * x * x))))


def _dot(a, b):
    return jnp.dot(a, b, preferred_element_type=F32)


def kernel(x_hbm, wqkv_hbm, wo_hbm, w1_hbm, b1_hbm, w2_hbm, b2_hbm, out_hbm,
           wqkv, wo, w1, w2, xin, xs, obuf, qkv, xn1, osc, acc_s, xn2_s, tmp, b1s, b2s, b1_ref, b2_ref,
           sem_x, sem_w, sem_f, sem_o):
    S, D = xin.shape
    G = D // 128
    NT = S // T
    NC = w1.shape[0]
    NU = 2 * NT

    def x_copy(t):
        return pltpu.make_async_copy(x_hbm.at[pl.ds(t * T, T), :], xin.at[pl.ds(t * T, T), :], sem_x.at[t])

    def wqkv_copy(j):
        return pltpu.make_async_copy(wqkv_hbm.at[:, pl.ds(j * D, D)], wqkv.at[j], sem_w.at[j])

    def wo_copy():
        return pltpu.make_async_copy(wo_hbm, wo, sem_w.at[3])

    def w1_copy(c):
        return pltpu.make_async_copy(w1_hbm.at[:, pl.ds(c * FC, FC)], w1.at[c], sem_f.at[2 * c])

    def w2_copy(c):
        return pltpu.make_async_copy(w2_hbm.at[pl.ds(c * FC, FC), :], w2.at[c], sem_f.at[2 * c + 1])

    def b_copies():
        return [pltpu.make_async_copy(b1_hbm, b1_ref, sem_w.at[4]), pltpu.make_async_copy(b2_hbm, b2_ref, sem_w.at[5])]

    def out_copy(t):
        return pltpu.make_async_copy(obuf.at[pl.ds(t * T, T), :], out_hbm.at[pl.ds(t * T, T), :], sem_o.at[t])

    stages = {
        2: 'x0 q|b|k x1|v o|f0 f1|f2 f3|f4 f5 f6 x2|xr',
        5: 'x0 q|x1 b|k|v|o f0|f1 f2 f3|f4 f5 f6 x2|xr',
        6: 'x0 q|b|k x1|v|o f0|f1 f2 f3|f4 f5 f6 x2|xr',
        7: 'x0 q|b|k x1|v o|f0|f1 f2 f3|f4 f5 f6 x2|xr',
        8: 'q x0|b|k x1|v o|f0 f1|f2 f3|f4 f5 f6 x2|xr',
        9: 'x0 q|b|x1 k|v o|f0 f1 f2 f3||f4 f5 f6 x2|xr',
    }[DQ].split('|')

    def issue(k):
        for nm in stages[k].split():
            if nm == 'b':
                cps = b_copies()
            elif nm == 'xr':
                cps = [x_copy(t) for t in range(3, NT)]
            elif nm[0] == 'x':
                cps = [x_copy(int(nm[1]))]
            elif nm[0] == 'f':
                cps = [w1_copy(int(nm[1])), w2_copy(int(nm[1]))]
            else:
                cps = [wo_copy() if nm == 'o' else wqkv_copy('qkv'.index(nm))]
            for cp in cps:
                cp.start()
    issue(0)

    def lanes(n):
        return lax.broadcasted_iota(jnp.int32, (n, 128), 1)

    def fold(t):
        parts = [t[a:a + 8, b:b + 128] for a in range(0, t.shape[0], 8) for b in range(0, t.shape[1], 128)]
        return functools.reduce(jnp.bitwise_or, parts)

    def pin(ref, toks, never):
        toks = [t for t in toks if t is not None]
        if toks and PIN:
            tok = pltpu.bitcast(functools.reduce(jnp.bitwise_or, toks), BF16)
            ref[0:16, 0:128] = jnp.where(never, tok, ref[0:16, 0:128])

    def shuffle_store(j, src, r0, n):
        lane = lanes(n)
        v = [src[pl.ds(r0, n), g * 128:(g + 1) * 128] for g in range(G)]
        for k in range(3):
            m = (lane & (4 << k)) != 0
            v = [jnp.where(m, v[(g + (1 << k)) % G], v[g]) for g in range(G)]
        for gp in range(G):
            idx = (lane & 3) * 32 + (((lane >> 2) - gp) & 7) * 4 + (lane >> 5)
            v[gp] = jnp.take_along_axis(v[gp], idx, axis=1)
            qkv[j, gp, pl.ds(HALO + r0, n), :] = v[gp]
        return fold(pltpu.bitcast(functools.reduce(jnp.maximum, v), U32))

    def load_x(u, r0, n):
        r = pl.multiple_of((u % NT) * T + r0, n)
        return jnp.where(u < NT, xin[pl.ds(r, n), :].astype(F32), xs[pl.ds(r, n), :])

    scale = DH ** -0.5

    def gate(x, link):
        if link is not None and link['tok'] is not None:
            return jnp.where(link['never'], link['tok'], x)
        return x

    def chain_sum(terms, link, serial):
        if link is None:
            return functools.reduce(lambda a, b: a + b, terms)
        if not serial:
            acc = functools.reduce(lambda a, b: a + b, terms[1:], gate(terms[0], link))
            link['tok'] = acc
            return acc
        parts = []
        if link['tok'] is not None:
            link['tok'] = link['tok'][RB - 8:RB]
        for a in range(0, RB, 8):
            acc = functools.reduce(lambda x, y: x + y, [t[a:a + 8] for t in terms[1:]], gate(terms[0][a:a + 8], link))
            link['tok'] = acc
            parts.append(acc)
        link['tok'] = jnp.concatenate([acc] * (RB // 8), axis=0)
        return jnp.concatenate(parts, axis=0)

    def attn_qk(tile, rb, link):
        r0 = HALO + rb * RB
        lg = []
        for w in range(W):
            acc = chain_sum([qkv[0, g, pl.ds(r0, RB), :] * qkv[1, g, pl.ds(r0 - DIL * w, RB), :]
                             for g in range(G)], link, w % SQ == 0 if SQ else False)
            acc = acc + pltpu.roll(acc, 32, 1)
            acc = acc + pltpu.roll(acc, 64, 1)
            acc = acc * scale
            if rb * RB < DIL * w:
                pos = tile * T + rb * RB + lax.broadcasted_iota(jnp.int32, (RB, 128), 0)
                acc = jnp.where(pos >= DIL * w, acc, -1e9)
            lg.append(acc)
        m = functools.reduce(jnp.maximum, lg)
        e = [jnp.exp(a - m) for a in lg]
        s = functools.reduce(lambda a, b: a + b, e)
        inv = 1.0 / s
        return [a * inv for a in e]

    def attn_pv(rb, p, link):
        r0 = HALO + rb * RB
        lane = lanes(RB // 2)
        o = []
        for gp in range(G):
            acc = chain_sum([p[w] * qkv[2, gp, pl.ds(r0 - DIL * w, RB), :] for w in range(W)],
                            link, gp % SP == 0 if SP else False)
            pk = pltpu.bitcast(acc.astype(BF16), U32)
            idx = (lane & 3) * 32 + (((lane >> 2) + gp) & 7) * 4 + (lane >> 5)
            o.append(jnp.take_along_axis(pk, idx, axis=1))
        for k in range(3):
            m = (lane & (4 << k)) != 0
            o = [jnp.where(m, o[(g - (1 << k)) % G], o[g]) for g in range(G)]
        osc[pl.ds(rb * RB // 2, RB // 2), :] = jnp.concatenate(o, axis=1)
        return pltpu.bitcast(o[0], F32)

    def attention(tile, never, lo=0, hi=T // RB):
        link = None if never is None else {'never': never, 'tok': None}
        ps = {}
        done = {}
        for i in range(lo, hi + AD):
            if i < hi:
                ps[i] = attn_qk(tile, i, link)
            if i >= lo + AD:
                j = i - AD
                if link is not None and j >= 2:
                    link['tok'] = jnp.maximum(link['tok'], jnp.concatenate([done[j - 2]] * (RB // 8), axis=0))
                done[j] = attn_pv(j, ps.pop(j), link)

    def ln_chain(load, dst, lb, dist, never):
        outs = []
        for t, r0 in enumerate(range(0, T, lb)):
            x = load(r0, lb)
            if t >= dist:
                x0 = jnp.where(never, outs[t - dist], x[0:8, 0:128])
                x = jnp.concatenate([jnp.concatenate([x0, x[0:8, 128:]], axis=1), x[8:]], axis=0)
            y = _ln(x).astype(BF16)
            dst[pl.ds(r0, lb), :] = y
            outs.append(pltpu.bitcast(fold(pltpu.bitcast(y, U32)), F32))
        return pltpu.bitcast(outs[-1], U32)

    def o_val():
        return pltpu.bitcast(osc[...], BF16)

    def interleave(mm, vp, ref, never, first, last):
        n = len(vp)
        dl = [first + (t * (last + 1 - first)) // n for t in range(n)]
        for i in range(len(mm) + 1):
            toks = [t() for t, d in zip(vp, dl) if d == i]
            if i < len(mm):
                pin(ref, toks, never)
                mm[i]()

    NP = D // PW

    def proj_piece(j, p):
        def f():
            tmp[j, :, p * PW:(p + 1) * PW] = _dot(xn1[...], wqkv[j, :, p * PW:(p + 1) * PW])
        return f

    def ffn_chunk(xn2, c):
        h = _dot(xn2, w1[c])
        h = _gelu(h + b1s[c]).astype(BF16)
        return _dot(h, w2[c])

    TH = T // 2
    qkv[:, :, 0:HALO, :] = jnp.zeros((3, G, HALO, 128), F32)
    acc_s[TH:T, :] = jnp.zeros((TH, D), F32)
    x_copy(0).wait()
    issue(1)
    xn2_s[...] = _ln(xin[0:T, :].astype(F32)).astype(BF16)

    def pro_body(j, carry):
        wqkv_copy(j).wait()
        for k in range(3):
            if stages[2 + k]:
                pl.when(j == k)(functools.partial(issue, 2 + k))

        @pl.when(j == 1)
        def _():
            x_copy(1).wait()
        jp = jnp.maximum(j - 1, 0)
        for r0 in range(TH, T, SB):
            shuffle_store(jp, acc_s, r0, SB)
        acc_s[0:TH, :] = _dot(xn2_s[0:TH, :], wqkv[j])
        src = pl.multiple_of((j + 1) * TH, TH)
        dst = pl.multiple_of(jp * TH, TH)
        xn1[pl.ds(dst, TH), :] = _ln(xin[pl.ds(src, TH), :].astype(F32)).astype(BF16)
        acc_s[TH:T, :] = _dot(xn2_s[TH:T, :], wqkv[j])
        for r0 in range(0, TH, SB):
            shuffle_store(j, acc_s, r0, SB)
        return carry
    lax.fori_loop(0, 3, pro_body, 0)
    issue(5)
    for cp in b_copies():
        cp.wait()
    for c in range(NC):
        b1s[c] = b1_ref[pl.ds(c * FC, FC)].astype(F32).reshape(1, FC)
    b2s[...] = b2_ref[...].astype(F32).reshape(1, D)
    for r0 in range(TH, T, SB):
        shuffle_store(2, acc_s, r0, SB)
    wo_copy().wait()

    def step(u, carry):
        tile = u % NT
        r = pl.multiple_of(tile * T, T)

        def wait_x():
            @pl.when(u + 2 < NT)
            def _():
                x_copy(u + 2).wait()
        if not XW:
            wait_x()

        never = u < 0
        pieces = [proj_piece(j, p) for j in range(3) for p in range(NP)]
        for f in pieces[:NPRE]:
            f()
        attention(tile, never)
        acc_s[...] = load_x(u, 0, T) + _dot(o_val(), wo[...])
        for f in pieces[NPRE:]:
            f()
        ln_chain(lambda r0, n: acc_s[pl.ds(r0, n), :], xn2_s, LB2, LD2, never)

        keep = (u + 1) % NT != 0
        u2 = jnp.minimum(u + 2, NU - 1)

        def halo(j):
            qkv[j, :, 0:HALO, :] = jnp.where(keep, qkv[j, :, T:T + HALO, :], 0.0)

        st = {'acc': None}

        def chunk(c):
            def f():
                if c in (0, WSPLIT):
                    @pl.when(u == 0)
                    def _():
                        for cc in (range(0, WSPLIT) if c == 0 else range(WSPLIT, NC)):
                            w1_copy(cc).wait()
                            w2_copy(cc).wait()
                        issue(6 if c == 0 else 7)
                    if XW and c == WSPLIT:
                        wait_x()
                if c == 0:
                    st['acc'] = acc_s[...] + b2s[...]
                st['acc'] = st['acc'] + ffn_chunk(xn2_s[...], c)
            return f
        tasks = ([functools.partial(halo, j) for j in (1, 2)]
                 + [functools.partial(shuffle_store, j, tmp.at[j], r0, SB) for j in range(3) for r0 in range(0, T, SB)]
                 + [functools.partial(ln_chain, functools.partial(load_x, u2), xn1, LB, LD, never)])
        interleave([chunk(c) for c in range(NC)], tasks, xn2_s, never, F0, NC - 1)
        xs[pl.ds(r, T), :] = st['acc']
        obuf[pl.ds(r, T), :] = st['acc'].astype(BF16)

        @pl.when(u >= NT)
        def _():
            out_copy(tile).start()
        return carry
    lax.fori_loop(0, NU - 1 if EPI else (NIT or NU), step, 0)
    if not EPI:
        for t in range(NIT + 2 if NIT else NT, NT):
            x_copy(t).wait()
        for t in range((NIT or NU) - NT):
            out_copy(t).wait()
        return

    nh = 2 if EP2 else 1
    for h in range(nh):
        n = T // nh
        attention(NT - 1, None, h * n // RB, (h + 1) * n // RB)
        x1 = xs[S - T + h * n:S - T + (h + 1) * n, :] + _dot(pltpu.bitcast(osc[h * n // 2:(h + 1) * n // 2, :], BF16), wo[...])
        xn2_s[h * n:(h + 1) * n, :] = _ln(x1).astype(BF16)
        acc_s[h * n:(h + 1) * n, :] = x1 + b2s[...]

    def epi_body(c, carry):
        acc_s[...] += ffn_chunk(xn2_s[...], c)
        return carry
    lax.fori_loop(0, NC, epi_body, 0)
    obuf[S - T:S, :] = acc_s[...].astype(BF16)
    out_copy(NT - 1).start()
    for t in range(NT):
        out_copy(t).wait()


@jax.jit
def pallas_interleave_layers__sliding_local_dilated__dense_activation_gelu__prompt_kernel(
        A_x, A_wqkv, A_wo, B_x, B_w1, B_b1, B_w2, B_b2):
    B, S, D = A_x.shape
    F = B_w1.shape[1]
    G = D // 128
    NC = F // FC
    NT = S // T
    hbm = pl.BlockSpec(memory_space=pl.ANY)
    out = pl.pallas_call(
        kernel,
        in_specs=[hbm] * 7,
        out_specs=hbm,
        out_shape=jax.ShapeDtypeStruct((S, D), A_x.dtype),
        scratch_shapes=[pltpu.VMEM((3, D, D), BF16),
                        pltpu.VMEM((D, D), BF16),
                        pltpu.VMEM((NC, D, FC), BF16),
                        pltpu.VMEM((NC, FC, D), BF16),
                        pltpu.VMEM((S, D), BF16),
                        pltpu.VMEM((S, D), F32),
                        pltpu.VMEM((S, D), BF16),
                        pltpu.VMEM((3, G, T + HALO, 128), F32),
                        pltpu.VMEM((T, D), BF16),
                        pltpu.VMEM((T // 2, D), U32),
                        pltpu.VMEM((T, D), F32),
                        pltpu.VMEM((T, D), BF16),
                        pltpu.VMEM((3, T, D), F32),
                        pltpu.VMEM((NC, 1, FC), F32),
                        pltpu.VMEM((1, D), F32),
                        pltpu.VMEM((F,), BF16),
                        pltpu.VMEM((D,), BF16),
                        pltpu.SemaphoreType.DMA((NT,)),
                        pltpu.SemaphoreType.DMA((6,)),
                        pltpu.SemaphoreType.DMA((2 * NC,)),
                        pltpu.SemaphoreType.DMA((NT,))],
        compiler_params=pltpu.CompilerParams(vmem_limit_bytes=100 * 1024 * 1024),
    )(A_x.reshape(S, D), A_wqkv, A_wo, B_w1, B_b1, B_w2, B_b2)
    return out.reshape(B, S, D)
```

```python
import functools
import jax
import jax.numpy as jnp
from jax import lax
import jax.experimental.pallas as pl
import jax.experimental.pallas.tpu as pltpu

T = 256
FC = 512
H = 32; DH = 32; W = 8; DIL = 2; HALO = 16
RB = 16
WSPLIT = 4
PW = 1024; SB = 32; LB = 16
PIN = 1
NPRE = 2; A0 = 7; L0 = 4; F0 = 2
CH = 1
AD = 1; LD = 1; LB2 = 32; LD2 = 1
SQ = 0; SP = 0
EPI = 1; NIT = 0
DQ = 13
EP2 = 1; XW = 1
DUM = 0
QG = 0
MG = 496; MP = 0; MO = 0
CB = 0; CM = 512
FX = 3; LG = 480; EPC = 1
QS = 1
SBT = 64; OS = 0
QK1 = 2
EPO = 0; EG = 0
F32 = jnp.float32; BF16 = jnp.bfloat16; U32 = jnp.uint32


def _ln(x):
    m = jnp.mean(x, axis=-1, keepdims=True)
    xc = x - m
    v = jnp.mean(xc * xc, axis=-1, keepdims=True)
    return xc * lax.rsqrt(v + 1e-5)


def _gelu(x):
    c = 0.7978845608028654
    return 0.5 * x * (1.0 + jnp.tanh(c * (x + 0.044715 * (x * x * x))))


def _dot(a, b):
    return jnp.dot(a, b, preferred_element_type=F32)


def kernel(x_hbm, wqkv_hbm, wo_hbm, w1_hbm, b1_hbm, w2_hbm, b2_hbm, out_hbm,
           wqkv, wo, w1, w2, xin, xs, obuf, qkv, xn1, osc, acc_s, xn2_s, tmp, b1s, b2s, b1_ref, b2_ref,
           sem_x, sem_w, sem_f, sem_o):
    S, D = xin.shape
    G = D // 128
    NT = S // T
    NC = b1s.shape[0]
    NXB = (NT - 2) // 2
    NU = 2 * NT

    def x_copy(t):
        return pltpu.make_async_copy(x_hbm.at[pl.ds(t * T, T), :], xin.at[pl.ds(t * T, T), :], sem_x.at[t])

    def wqkv_copy(j):
        n = D // QS
        return [pltpu.make_async_copy(wqkv_hbm.at[pl.ds(i * n, n), pl.ds(j * D, D)], wqkv.at[j, pl.ds(i * n, n), :],
                                      sem_w.at[3 + j * QS + i]) for i in range(QS)]

    def wo_copy():
        return pltpu.make_async_copy(wo_hbm, wo, sem_w.at[0])

    def xb_copy(k):
        rows = pl.ds(pl.multiple_of((2 + k * NXB) * T, T), NXB * T)
        return pltpu.make_async_copy(x_hbm.at[rows, :], xin.at[rows, :], sem_x.at[2 + k])

    def ffn_copies(k):
        lo, hi = (0, WSPLIT * FC) if k == 0 else (WSPLIT * FC, NC * FC)
        return [pltpu.make_async_copy(w1_hbm.at[:, pl.ds(lo, hi - lo)], w1.at[:, pl.ds(lo, hi - lo)], sem_f.at[2 * k]),
                pltpu.make_async_copy(w2_hbm.at[pl.ds(lo, hi - lo), :], w2.at[pl.ds(lo, hi - lo), :], sem_f.at[2 * k + 1])]

    def b_copies():
        return [pltpu.make_async_copy(b1_hbm, b1_ref, sem_w.at[1]), pltpu.make_async_copy(b2_hbm, b2_ref, sem_w.at[2])]

    def out_copy(t):
        return pltpu.make_async_copy(obuf.at[pl.ds(t * T, T), :], out_hbm.at[pl.ds(t * T, T), :], sem_o.at[t])

    stages = {
        9: 'x0 q|b|x1 k|v o|f0||f1 y0|y1',
        13: 'x0 q|b x1|k|v o|f0||f1 y0|y1',
        14: 'x0 q|b|x1 k|v o|f0|y0|f1|y1',
    }[DQ].split('|')

    def issue(k):
        for nm in stages[k].split():
            if nm == 'b':
                cps = b_copies()
            elif nm[0] == 'y':
                cps = [xb_copy(int(nm[1]))]
            elif nm[0] == 'x':
                cps = [x_copy(int(nm[1]))]
            elif nm[0] == 'f':
                cps = ffn_copies(int(nm[1]))
            else:
                cps = [wo_copy()] if nm == 'o' else wqkv_copy('qkv'.index(nm))
            for cp in cps:
                cp.start()
    issue(0)

    def lanes(n):
        return lax.broadcasted_iota(jnp.int32, (n, 128), 1)

    def fold(t):
        parts = [t[a:a + 8, b:b + 128] for a in range(0, t.shape[0], 8) for b in range(0, t.shape[1], 128)]
        return functools.reduce(jnp.bitwise_or, parts)

    def pin(ref, toks, never):
        toks = [t for t in toks if t is not None]
        if toks and PIN:
            tok = pltpu.bitcast(functools.reduce(jnp.bitwise_or, toks), BF16)
            ref[0:16, 0:128] = jnp.where(never, tok, ref[0:16, 0:128])

    def shuffle_store(j, src, r0, n):
        lane = lanes(n)
        v = [src[pl.ds(r0, n), g * 128:(g + 1) * 128] for g in range(G)]
        for k in range(3):
            m = (lane & (4 << k)) != 0
            v = [jnp.where(m, v[(g + (1 << k)) % G], v[g]) for g in range(G)]
        for gp in range(G):
            idx = (lane & 3) * 32 + (((lane >> 2) - gp) & 7) * 4 + (lane >> 5)
            v[gp] = jnp.take_along_axis(v[gp], idx, axis=1)
            qkv[j, gp, pl.ds(HALO + r0, n), :] = v[gp]
        return fold(pltpu.bitcast(functools.reduce(jnp.maximum, v), U32))

    def load_x(u, r0, n):
        r = pl.multiple_of((u % NT) * T + r0, n)
        return jnp.where(u < NT, xin[pl.ds(r, n), :].astype(F32), xs[pl.ds(r, n), :])

    scale = DH ** -0.5

    def gate(x, link):
        if link is not None and link['tok'] is not None:
            return jnp.where(link['never'], link['tok'], x)
        return x

    def chain_sum(terms, link, serial):
        if link is None:
            return functools.reduce(lambda a, b: a + b, terms)
        if not serial:
            acc = functools.reduce(lambda a, b: a + b, terms[1:], gate(terms[0], link))
            tok = acc
            if DUM:
                tok = functools.reduce(jnp.maximum, [acc[a:a + 8] for a in range(0, RB, 8)])
                for i in range(DUM - 1):
                    tok = tok * 1.5 if i % 2 else tok + 1.0
                tok = jnp.concatenate([tok] * (RB // 8), axis=0)
            link['tok'] = tok
            return acc
        parts = []
        if link['tok'] is not None:
            link['tok'] = link['tok'][RB - 8:RB]
        for a in range(0, RB, 8):
            acc = functools.reduce(lambda x, y: x + y, [t[a:a + 8] for t in terms[1:]], gate(terms[0][a:a + 8], link))
            link['tok'] = acc
            parts.append(acc)
        link['tok'] = jnp.concatenate([acc] * (RB // 8), axis=0)
        return jnp.concatenate(parts, axis=0)

    def attn_qk(tile, rb, link):
        r0 = HALO + rb * RB
        lg = []
        accs = [None] * W
        if QG:
            for g in range(G):
                q = gate(qkv[0, g, pl.ds(r0, RB), :], link)
                for w in range(W):
                    t = q * qkv[1, g, pl.ds(r0 - DIL * w, RB), :]
                    accs[w] = t if g == 0 else accs[w] + t
                if link is not None:
                    tok = accs[0][0:8]
                    for i in range(1, QG):
                        tok = jnp.maximum(tok, accs[i % W][8 * (i % 2):8 * (i % 2) + 8])
                    link['tok'] = jnp.concatenate([tok] * (RB // 8), axis=0)
        for w in range(W):
            acc = accs[w] if QG else chain_sum(
                [qkv[0, g, pl.ds(r0, RB), :] * qkv[1, g, pl.ds(r0 - DIL * w, RB), :]
                 for g in range(G)], link, w % SQ == 0 if SQ else False)
            acc = acc + pltpu.roll(acc, 32, 1)
            acc = acc + pltpu.roll(acc, 64, 1)
            if not FX:
                acc = acc * scale
            if rb * RB < DIL * w:
                pos = tile * T + rb * RB + lax.broadcasted_iota(jnp.int32, (RB, 128), 0)
                acc = jnp.where(pos >= DIL * w, acc, -1e9 / scale if FX else -1e9)
            lg.append(acc)
        m = functools.reduce(jnp.maximum, lg)
        if FX:
            e = [jnp.exp2((a - m) * (scale * 1.4426950408889634)) for a in lg]
        else:
            e = [jnp.exp(a - m) for a in lg]
        s = functools.reduce(lambda a, b: a + b, e)
        if FX & 2:
            inv = pl.reciprocal(s, approx=True)
            inv = inv * (2.0 - s * inv)
        else:
            inv = 1.0 / s
        return [a * inv for a in e]

    def attn_pv(rb, p, link):
        r0 = HALO + rb * RB
        lane = lanes(RB // 2)
        o = []
        for gp in range(G):
            acc = chain_sum([p[w] * qkv[2, gp, pl.ds(r0 - DIL * w, RB), :] for w in range(W)],
                            link, gp % SP == 0 if SP else False)
            pk = pltpu.bitcast(acc.astype(BF16), U32)
            idx = (lane & 3) * 32 + (((lane >> 2) + gp) & 7) * 4 + (lane >> 5)
            o.append(jnp.take_along_axis(pk, idx, axis=1))
        for k in range(3):
            m = (lane & (4 << k)) != 0
            o = [jnp.where(m, o[(g - (1 << k)) % G], o[g]) for g in range(G)]
        osc[pl.ds(rb * RB // 2, RB // 2), :] = jnp.concatenate(o, axis=1)
        return pltpu.bitcast(o[0], F32)

    def attention(tile, never, lo=0, hi=T // RB, clock=None, mg=MG):
        link = None if never is None else {'never': never, 'tok': None}
        ps = {}
        done = {}
        for i in range(lo, hi + AD):
            if clock is not None and clock((i - lo) * mg) is not None:
                link['tok'] = jnp.maximum(link['tok'], clock((i - lo) * mg))
            if i < hi:
                ps[i] = attn_qk(tile, i, link)
            if i >= lo + AD:
                j = i - AD
                if link is not None and j >= lo + 2:
                    link['tok'] = jnp.maximum(link['tok'], jnp.concatenate([done[j - 2]] * (RB // 8), axis=0))
                done[j] = attn_pv(j, ps.pop(j), link)

    def mm_clock(res, n, t):
        m = res.shape[0]
        t = min(t, res.shape[1] // 128 * 2 * m)
        c, o = t // (2 * m), t % (2 * m) - m
        if o < 0:
            c, o = c - 1, m - n
        o = o // n * n
        return res[o:o + n, c * 128:(c + 1) * 128] if c >= 0 else None

    def ln_chain(load, dst, lb, dist, never, clock=None):
        outs = []
        for t, r0 in enumerate(range(0, T, lb)):
            x = load(r0, lb)
            if t >= dist:
                tok = outs[t - dist]
                if clock is not None and clock(t * LG) is not None:
                    tok = jnp.maximum(tok, clock(t * LG))
                x0 = jnp.where(never, tok, x[0:8, 0:128])
                x = jnp.concatenate([jnp.concatenate([x0, x[0:8, 128:]], axis=1), x[8:]], axis=0)
            y = _ln(x).astype(BF16)
            dst[pl.ds(r0, lb), :] = y
            outs.append(pltpu.bitcast(fold(pltpu.bitcast(y, U32)), F32))
        return pltpu.bitcast(outs[-1], U32)

    def o_val():
        return pltpu.bitcast(osc[...], BF16)

    def interleave(mm, vp, ref, never, first, last):
        n = len(vp)
        dl = [first + (t * (last + 1 - first)) // n for t in range(n)]
        for i in range(len(mm) + 1):
            toks = [t() for t, d in zip(vp, dl) if d == i]
            if i < len(mm):
                pin(ref, toks, never)
                mm[i]()

    NP = D // PW

    def proj_piece(j, p):
        def f():
            res = _dot(xn1[...], wqkv[j, :, p * PW:(p + 1) * PW])
            tmp[j, :, p * PW:(p + 1) * PW] = res
            return res
        return f

    def ffn_chunk(xn2, c, mid=None):
        cols = pl.ds(c * FC if isinstance(c, int) else pl.multiple_of(c * FC, FC), FC)
        h = _dot(xn2, w1[:, cols])
        if mid is not None:
            mid(h)
        h = _gelu(h + b1s[c]).astype(BF16)
        return _dot(h, w2[cols, :])

    TH = T // 2
    qkv[:, :, 0:HALO, :] = jnp.zeros((3, G, HALO, 128), F32)
    acc_s[TH:T, :] = jnp.zeros((TH, D), F32)
    x_copy(0).wait()
    issue(1)
    xn2_s[...] = _ln(xin[0:T, :].astype(F32)).astype(BF16)

    def pro_body(j, carry):
        for cp in wqkv_copy(j):
            cp.wait()
        for k in range(3):
            if stages[2 + k]:
                pl.when(j == k)(functools.partial(issue, 2 + k))

        @pl.when(j == 1)
        def _():
            x_copy(1).wait()
        jp = jnp.maximum(j - 1, 0)
        for r0 in range(TH, T, SB):
            shuffle_store(jp, acc_s, r0, SB)
        acc_s[0:TH, :] = _dot(xn2_s[0:TH, :], wqkv[j])
        src = pl.multiple_of((j + 1) * TH, TH)
        dst = pl.multiple_of(jp * TH, TH)
        xn1[pl.ds(dst, TH), :] = _ln(xin[pl.ds(src, TH), :].astype(F32)).astype(BF16)
        acc_s[TH:T, :] = _dot(xn2_s[TH:T, :], wqkv[j])
        for r0 in range(0, TH, SB):
            shuffle_store(j, acc_s, r0, SB)
        return carry
    lax.fori_loop(0, 3, pro_body, 0)
    issue(5)
    for cp in b_copies():
        cp.wait()
    for c in range(NC):
        b1s[c] = b1_ref[pl.ds(c * FC, FC)].astype(F32).reshape(1, FC)
    b2s[...] = b2_ref[...].astype(F32).reshape(1, D)
    for r0 in range(TH, T, SBT):
        shuffle_store(2, acc_s, r0, SBT)
    wo_copy().wait()

    def step(u, carry):
        tile = u % NT
        r = pl.multiple_of(tile * T, T)

        never = u < 0
        pieces = [proj_piece(j, p) for j in range(3) for p in range(NP)]
        if QK1:
            xn1v = xn1[...]
            pre = _dot(xn1v, jnp.concatenate([wqkv[0], wqkv[1]], axis=1))
            tmp[0] = pre[:, 0:D]
            tmp[1] = pre[:, D:2 * D]
        else:
            pre = jnp.concatenate([f() for f in pieces[:NPRE]], axis=1)

        clock = functools.partial(mm_clock, pre, RB) if MG else None
        attention(tile, never, clock=clock)
        acc_s[...] = load_x(u, 0, T) + _dot(o_val(), wo[...])

        def barrier(k):
            @pl.when(u == 0)
            def _():
                for cp in ffn_copies(k):
                    cp.wait()
                issue(6 + k)
            if k == 1:
                @pl.when(u < 2)
                def _():
                    xb_copy(jnp.minimum(u, 1)).wait()

        res = _dot(xn1v, wqkv[2])
        tmp[2] = res
        ln_chain(lambda r0, n: acc_s[pl.ds(r0, n), :], xn2_s, LB2, LD2, never, functools.partial(mm_clock, res, 8))

        keep = (u + 1) % NT != 0
        u2 = jnp.minimum(u + 2, NU - 1)

        def halo(j):
            qkv[j, :, 0:HALO, :] = jnp.where(keep, qkv[j, :, T:T + HALO, :], 0.0)

        st = {'acc': None}

        def chunk(c):
            def f():
                if c == 0:
                    barrier(0)
                if c == WSPLIT:
                    barrier(1)
                if c == 0:
                    st['acc'] = acc_s[...] + b2s[...]
                st['acc'] = st['acc'] + ffn_chunk(xn2_s[...], c)
            return f
        tasks = ([functools.partial(halo, j) for j in (1, 2)]
                 + [functools.partial(shuffle_store, j, tmp.at[j], r0, SB) for j in range(3) for r0 in range(0, T, SB)]
                 + [functools.partial(ln_chain, functools.partial(load_x, u2), xn1, LB, LD, never)])
        interleave([chunk(c) for c in range(NC)], tasks, xn2_s, never, F0, NC - 1)
        xs[pl.ds(r, T), :] = st['acc']
        obuf[pl.ds(r, T), :] = st['acc'].astype(BF16)

        @pl.when(u >= NT)
        def _():
            out_copy(tile).start()
        return u
    last = lax.fori_loop(0, NU - 1 if EPI else (NIT or NU), step, 0)
    if not EPI:
        for t in range((NIT or NU) - NT):
            out_copy(t).wait()
        return

    def epi_wo(h):
        y = _dot(pltpu.bitcast(osc[h * TH // 2:(h + 1) * TH // 2, :], BF16), wo[...])
        x1 = xs[S - T + h * TH:S - T + (h + 1) * TH, :] + y
        xn2_s[h * TH:(h + 1) * TH, :] = _ln(x1).astype(BF16)
        acc_s[h * TH:(h + 1) * TH, :] = x1 + b2s[...]
        return y

    def epi_second(y0):
        if EG:
            attention(NT - 1, last < 0, TH // RB, T // RB, functools.partial(mm_clock, y0, RB), EG)
        else:
            attention(NT - 1, None, TH // RB, T // RB)
        epi_wo(1)

    attention(NT - 1, None, 0, TH // RB)
    y0 = epi_wo(0)
    if EPO:
        acc_s[0:TH, :] += ffn_chunk(xn2_s[0:TH, :], 0, lambda h: epi_second(jnp.concatenate([y0, h], axis=1)))
    else:
        epi_second(y0)
        acc_s[0:TH, :] += ffn_chunk(xn2_s[0:TH, :], 0)
    acc_s[TH:T, :] += ffn_chunk(xn2_s[TH:T, :], 0)

    def epi_body(c, carry):
        a = acc_s[...] + ffn_chunk(xn2_s[...], c)
        acc_s[...] = a
        obuf[S - T:S, :] = a.astype(BF16)
        return carry
    lax.fori_loop(1, NC, epi_body, 0)
    out_copy(NT - 1).start()
    for t in range(NT):
        out_copy(t).wait()


@jax.jit
def pallas_interleave_layers__sliding_local_dilated__dense_activation_gelu__prompt_kernel(
        A_x, A_wqkv, A_wo, B_x, B_w1, B_b1, B_w2, B_b2):
    B, S, D = A_x.shape
    F = B_w1.shape[1]
    G = D // 128
    NC = F // FC
    NT = S // T
    hbm = pl.BlockSpec(memory_space=pl.ANY)
    out = pl.pallas_call(
        kernel,
        in_specs=[hbm] * 7,
        out_specs=hbm,
        out_shape=jax.ShapeDtypeStruct((S, D), A_x.dtype),
        scratch_shapes=[pltpu.VMEM((3, D, D), BF16),
                        pltpu.VMEM((D, D), BF16),
                        pltpu.VMEM((D, F), BF16),
                        pltpu.VMEM((F, D), BF16),
                        pltpu.VMEM((S, D), BF16),
                        pltpu.VMEM((S, D), F32),
                        pltpu.VMEM((S, D), BF16),
                        pltpu.VMEM((3, G, T + HALO, 128), F32),
                        pltpu.VMEM((T, D), BF16),
                        pltpu.VMEM((T // 2, D), U32),
                        pltpu.VMEM((T, D), F32),
                        pltpu.VMEM((T, D), BF16),
                        pltpu.VMEM((3, T, D), F32),
                        pltpu.VMEM((NC, 1, FC), F32),
                        pltpu.VMEM((1, D), F32),
                        pltpu.VMEM((F,), BF16),
                        pltpu.VMEM((D,), BF16),
                        pltpu.SemaphoreType.DMA((4,)),
                        pltpu.SemaphoreType.DMA((3 + 3 * QS,)),
                        pltpu.SemaphoreType.DMA((4,)),
                        pltpu.SemaphoreType.DMA((NT,))],
        compiler_params=pltpu.CompilerParams(vmem_limit_bytes=100 * 1024 * 1024),
    )(A_x.reshape(S, D), A_wqkv, A_wo, B_w1, B_b1, B_w2, B_b2)
    return out.reshape(B, S, D)
```

```python
import functools
import jax
import jax.numpy as jnp
from jax import lax
import jax.experimental.pallas as pl
import jax.experimental.pallas.tpu as pltpu

T = 256
FC = 512
DH = 32; W = 8; DIL = 2; HALO = 16
RB = 16
WSPLIT = 4
PW = 1024; SB = 16; LB = 16
PIN = 1
NPRE = 2; F0 = 2
AD = 1; LD = 2; LB2 = 32; LD2 = 1
SQ = 0; SP = 0
DUM = 0
QG = 0
MG = 496
FX = 3; LG = 480
SBT = 64
QK1 = 2
EPO = 0; EG = 0
XS = 1; XI = 0
F32 = jnp.float32; BF16 = jnp.bfloat16; U32 = jnp.uint32


def _ln(x):
    m = jnp.mean(x, axis=-1, keepdims=True)
    xc = x - m
    v = jnp.mean(xc * xc, axis=-1, keepdims=True)
    return xc * lax.rsqrt(v + 1e-5)


def _gelu(x):
    c = 0.7978845608028654
    return 0.5 * x * (1.0 + jnp.tanh(c * (x + 0.044715 * (x * x * x))))


def _dot(a, b):
    return jnp.dot(a, b, preferred_element_type=F32)


def kernel(x_hbm, wqkv_hbm, wo_hbm, w1_hbm, b1_hbm, w2_hbm, b2_hbm, out_hbm,
           wqkv, wo, w1, w2, xin, xs, obuf, qkv, xn1, osc, acc_s, xn2_s, tmp, b1s, b2s, b1_ref, b2_ref,
           sem_x, sem_w, sem_f, sem_o):
    S, D = xin.shape
    G = D // 128
    NT = S // T
    NC = b1s.shape[0]
    NXB = (NT - 2) // 2
    NU = 2 * NT

    def x_copy(t):
        return pltpu.make_async_copy(x_hbm.at[pl.ds(t * T, T), :], xin.at[pl.ds(t * T, T), :], sem_x.at[t])

    DH2 = D // 2

    def wqkv_copy(j, i):
        return pltpu.make_async_copy(wqkv_hbm.at[:, pl.ds(pl.multiple_of(j * D + i * DH2, DH2), DH2)],
                                     wqkv.at[j, :, pl.ds(i * DH2, DH2)], sem_w.at[3 + 2 * j + i])

    def wo_copy():
        return pltpu.make_async_copy(wo_hbm, wo, sem_w.at[0])

    def x0_copy(i):
        rows = pl.ds(i * (T // XS), T // XS)
        return pltpu.make_async_copy(x_hbm.at[rows, :], xin.at[rows, :], sem_x.at[4 + i])

    def xb_copy(k):
        rows = pl.ds(pl.multiple_of((2 + k * NXB) * T, T), NXB * T)
        return pltpu.make_async_copy(x_hbm.at[rows, :], xin.at[rows, :], sem_x.at[2 + k])

    def ffn_copies(k):
        lo, hi = (0, WSPLIT * FC) if k == 0 else (WSPLIT * FC, NC * FC)
        return [pltpu.make_async_copy(w1_hbm.at[:, pl.ds(lo, hi - lo)], w1.at[:, pl.ds(lo, hi - lo)], sem_f.at[2 * k]),
                pltpu.make_async_copy(w2_hbm.at[pl.ds(lo, hi - lo), :], w2.at[pl.ds(lo, hi - lo), :], sem_f.at[2 * k + 1])]

    def b_copies():
        return [pltpu.make_async_copy(b1_hbm, b1_ref, sem_w.at[1]), pltpu.make_async_copy(b2_hbm, b2_ref, sem_w.at[2])]

    def out_copy(t):
        return pltpu.make_async_copy(obuf.at[pl.ds(t * T, T), :], out_hbm.at[pl.ds(t * T, T), :], sem_o.at[t])

    stages = 'x0 q0|q1|k0 x1|k1|v0|v1 b|o|f0||f1 y0|y1'.split('|')

    def issue(k):
        for nm in stages[k].split():
            if nm == 'b':
                cps = b_copies()
            elif nm[0] == 'y':
                cps = [xb_copy(int(nm[1]))]
            elif nm == 'x0':
                cps = [x0_copy(i) for i in range(XS)]
            elif nm[0] == 'x':
                cps = [x_copy(int(nm[1]))]
            elif nm[0] == 'f':
                cps = ffn_copies(int(nm[1]))
            else:
                cps = [wo_copy() if nm == 'o' else wqkv_copy('qkv'.index(nm[0]), int(nm[1]))]
            for cp in cps:
                cp.start()
    issue(0)

    def lanes(n):
        return lax.broadcasted_iota(jnp.int32, (n, 128), 1)

    def fold(t):
        parts = [t[a:a + 8, b:b + 128] for a in range(0, t.shape[0], 8) for b in range(0, t.shape[1], 128)]
        return functools.reduce(jnp.bitwise_or, parts)

    def pin(ref, toks, never):
        toks = [t for t in toks if t is not None]
        if toks and PIN:
            tok = pltpu.bitcast(functools.reduce(jnp.bitwise_or, toks), BF16)
            ref[0:16, 0:128] = jnp.where(never, tok, ref[0:16, 0:128])

    def shuffle_store(j, src, r0, n):
        lane = lanes(n)
        v = [src[pl.ds(r0, n), g * 128:(g + 1) * 128] for g in range(G)]
        for k in range(3):
            m = (lane & (4 << k)) != 0
            v = [jnp.where(m, v[(g + (1 << k)) % G], v[g]) for g in range(G)]
        for gp in range(G):
            idx = (lane & 3) * 32 + (((lane >> 2) - gp) & 7) * 4 + (lane >> 5)
            v[gp] = jnp.take_along_axis(v[gp], idx, axis=1)
            qkv[j, gp, pl.ds(HALO + r0, n), :] = v[gp]
        return fold(pltpu.bitcast(functools.reduce(jnp.maximum, v), U32))

    def load_x(u, r0, n):
        r = pl.multiple_of((u % NT) * T + r0, n)
        return jnp.where(u < NT, xin[pl.ds(r, n), :].astype(F32), xs[pl.ds(r, n), :])

    scale = DH ** -0.5

    def gate(x, link):
        if link is not None and link['tok'] is not None:
            return jnp.where(link['never'], link['tok'], x)
        return x

    def chain_sum(terms, link, serial):
        if link is None:
            return functools.reduce(lambda a, b: a + b, terms)
        if not serial:
            acc = functools.reduce(lambda a, b: a + b, terms[1:], gate(terms[0], link))
            tok = acc
            if DUM:
                tok = functools.reduce(jnp.maximum, [acc[a:a + 8] for a in range(0, RB, 8)])
                for i in range(DUM - 1):
                    tok = tok * 1.5 if i % 2 else tok + 1.0
                tok = jnp.concatenate([tok] * (RB // 8), axis=0)
            link['tok'] = tok
            return acc
        parts = []
        if link['tok'] is not None:
            link['tok'] = link['tok'][RB - 8:RB]
        for a in range(0, RB, 8):
            acc = functools.reduce(lambda x, y: x + y, [t[a:a + 8] for t in terms[1:]], gate(terms[0][a:a + 8], link))
            link['tok'] = acc
            parts.append(acc)
        link['tok'] = jnp.concatenate([acc] * (RB // 8), axis=0)
        return jnp.concatenate(parts, axis=0)

    def attn_qk(tile, rb, link):
        r0 = HALO + rb * RB
        lg = []
        accs = [None] * W
        if QG:
            for g in range(G):
                q = gate(qkv[0, g, pl.ds(r0, RB), :], link)
                for w in range(W):
                    t = q * qkv[1, g, pl.ds(r0 - DIL * w, RB), :]
                    accs[w] = t if g == 0 else accs[w] + t
                if link is not None:
                    tok = accs[0][0:8]
                    for i in range(1, QG):
                        tok = jnp.maximum(tok, accs[i % W][8 * (i % 2):8 * (i % 2) + 8])
                    link['tok'] = jnp.concatenate([tok] * (RB // 8), axis=0)
        for w in range(W):
            acc = accs[w] if QG else chain_sum(
                [qkv[0, g, pl.ds(r0, RB), :] * qkv[1, g, pl.ds(r0 - DIL * w, RB), :]
                 for g in range(G)], link, w % SQ == 0 if SQ else False)
            acc = acc + pltpu.roll(acc, 32, 1)
            acc = acc + pltpu.roll(acc, 64, 1)
            if not FX:
                acc = acc * scale
            if rb * RB < DIL * w:
                pos = tile * T + rb * RB + lax.broadcasted_iota(jnp.int32, (RB, 128), 0)
                acc = jnp.where(pos >= DIL * w, acc, -1e9 / scale if FX else -1e9)
            lg.append(acc)
        m = functools.reduce(jnp.maximum, lg)
        if FX:
            e = [jnp.exp2((a - m) * (scale * 1.4426950408889634)) for a in lg]
        else:
            e = [jnp.exp(a - m) for a in lg]
        s = functools.reduce(lambda a, b: a + b, e)
        if FX & 2:
            inv = pl.reciprocal(s, approx=True)
            inv = inv * (2.0 - s * inv)
        else:
            inv = 1.0 / s
        return [a * inv for a in e]

    def attn_pv(rb, p, link):
        r0 = HALO + rb * RB
        lane = lanes(RB // 2)
        o = []
        for gp in range(G):
            acc = chain_sum([p[w] * qkv[2, gp, pl.ds(r0 - DIL * w, RB), :] for w in range(W)],
                            link, gp % SP == 0 if SP else False)
            pk = pltpu.bitcast(acc.astype(BF16), U32)
            idx = (lane & 3) * 32 + (((lane >> 2) + gp) & 7) * 4 + (lane >> 5)
            o.append(jnp.take_along_axis(pk, idx, axis=1))
        for k in range(3):
            m = (lane & (4 << k)) != 0
            o = [jnp.where(m, o[(g - (1 << k)) % G], o[g]) for g in range(G)]
        osc[pl.ds(rb * RB // 2, RB // 2), :] = jnp.concatenate(o, axis=1)
        return pltpu.bitcast(o[0], F32)

    def attention(tile, never, lo=0, hi=T // RB, clock=None, mg=MG):
        link = None if never is None else {'never': never, 'tok': None}
        ps = {}
        done = {}
        for i in range(lo, hi + AD):
            if clock is not None and clock((i - lo) * mg) is not None:
                link['tok'] = jnp.maximum(link['tok'], clock((i - lo) * mg))
            if i < hi:
                ps[i] = attn_qk(tile, i, link)
            if i >= lo + AD:
                j = i - AD
                if link is not None and j >= lo + 2:
                    link['tok'] = jnp.maximum(link['tok'], jnp.concatenate([done[j - 2]] * (RB // 8), axis=0))
                done[j] = attn_pv(j, ps.pop(j), link)

    def mm_clock(res, n, t):
        m = res.shape[0]
        t = min(t, res.shape[1] // 128 * 2 * m)
        c, o = t // (2 * m), t % (2 * m) - m
        if o < 0:
            c, o = c - 1, m - n
        o = o // n * n
        return res[o:o + n, c * 128:(c + 1) * 128] if c >= 0 else None

    def ln_chain(load, dst, lb, dist, never, clock=None):
        outs = []
        for t, r0 in enumerate(range(0, T, lb)):
            x = load(r0, lb)
            if t >= dist:
                tok = outs[t - dist]
                if clock is not None and clock(t * LG) is not None:
                    tok = jnp.maximum(tok, clock(t * LG))
                x0 = jnp.where(never, tok, x[0:8, 0:128])
                x = jnp.concatenate([jnp.concatenate([x0, x[0:8, 128:]], axis=1), x[8:]], axis=0)
            y = _ln(x).astype(BF16)
            dst[pl.ds(r0, lb), :] = y
            outs.append(pltpu.bitcast(fold(pltpu.bitcast(y, U32)), F32))
        return pltpu.bitcast(outs[-1], U32)

    def o_val():
        return pltpu.bitcast(osc[...], BF16)

    def interleave(mm, vp, ref, never, first, last):
        n = len(vp)
        dl = [first + (t * (last + 1 - first)) // n for t in range(n)]
        for i in range(len(mm) + 1):
            toks = [t() for t, d in zip(vp, dl) if d == i]
            if i < len(mm):
                pin(ref, toks, never)
                mm[i]()

    NP = D // PW

    def proj_piece(j, p):
        def f():
            res = _dot(xn1[...], wqkv[j, :, p * PW:(p + 1) * PW])
            tmp[j, :, p * PW:(p + 1) * PW] = res
            return res
        return f

    def ffn_chunk(xn2, c, mid=None):
        cols = pl.ds(c * FC if isinstance(c, int) else pl.multiple_of(c * FC, FC), FC)
        h = _dot(xn2, w1[:, cols])
        if mid is not None:
            mid(h)
        h = _gelu(h + b1s[c]).astype(BF16)
        return _dot(h, w2[cols, :])

    TH = T // 2
    qkv[:, :, 0:HALO, :] = jnp.zeros((3, G, HALO, 128), F32)
    acc_s[TH:T, :] = jnp.zeros((TH, D), F32)
    for i in range(XS):
        x0_copy(i).wait()
        if i == XI:
            issue(1)
        rows = pl.ds(i * (T // XS), T // XS)
        xn2_s[rows, :] = _ln(xin[rows, :].astype(F32)).astype(BF16)

    def pro_body(j, carry):
        def arrive(i):
            wqkv_copy(j, i).wait()
            for k in range(3):
                if stages[2 + 2 * k + i]:
                    pl.when(j == k)(functools.partial(issue, 2 + 2 * k + i))
        jp = jnp.maximum(j - 1, 0)
        arrive(0)
        for r0 in range(TH, T, SB):
            shuffle_store(jp, acc_s, r0, SB)
        for h in range(2):
            acc_s[h * TH:(h + 1) * TH, 0:DH2] = _dot(xn2_s[h * TH:(h + 1) * TH, :], wqkv[j, :, 0:DH2])
        arrive(1)

        @pl.when(j == 1)
        def _():
            x_copy(1).wait()
        src = pl.multiple_of((j + 1) * TH, TH)
        dst = pl.multiple_of(jp * TH, TH)
        xn1[pl.ds(dst, TH), :] = _ln(xin[pl.ds(src, TH), :].astype(F32)).astype(BF16)
        for h in range(2):
            acc_s[h * TH:(h + 1) * TH, DH2:D] = _dot(xn2_s[h * TH:(h + 1) * TH, :], wqkv[j, :, DH2:D])
        for r0 in range(0, TH, SB):
            shuffle_store(j, acc_s, r0, SB)
        return carry
    lax.fori_loop(0, 3, pro_body, 0)
    issue(8)
    for cp in b_copies():
        cp.wait()
    for c in range(NC):
        b1s[c] = b1_ref[pl.ds(c * FC, FC)].astype(F32).reshape(1, FC)
    b2s[...] = b2_ref[...].astype(F32).reshape(1, D)
    for r0 in range(TH, T, SBT):
        shuffle_store(2, acc_s, r0, SBT)
    wo_copy().wait()

    def step(u, carry):
        tile = u % NT
        r = pl.multiple_of(tile * T, T)

        never = u < 0
        pieces = [proj_piece(j, p) for j in range(3) for p in range(NP)]
        if QK1:
            xn1v = xn1[...]
            pre = _dot(xn1v, jnp.concatenate([wqkv[0], wqkv[1]], axis=1))
            tmp[0] = pre[:, 0:D]
            tmp[1] = pre[:, D:2 * D]
        else:
            pre = jnp.concatenate([f() for f in pieces[:NPRE]], axis=1)

        clock = functools.partial(mm_clock, pre, RB) if MG else None
        attention(tile, never, clock=clock)
        acc_s[...] = load_x(u, 0, T) + _dot(o_val(), wo[...])

        def barrier(k):
            @pl.when(u == 0)
            def _():
                for cp in ffn_copies(k):
                    cp.wait()
                issue(9 + k)
            if k == 1:
                @pl.when(u < 2)
                def _():
                    xb_copy(jnp.minimum(u, 1)).wait()

        res = _dot(xn1v, wqkv[2])
        tmp[2] = res
        ln_chain(lambda r0, n: acc_s[pl.ds(r0, n), :], xn2_s, LB2, LD2, never, functools.partial(mm_clock, res, 8))

        keep = (u + 1) % NT != 0
        u2 = jnp.minimum(u + 2, NU - 1)

        def halo(j):
            qkv[j, :, 0:HALO, :] = jnp.where(keep, qkv[j, :, T:T + HALO, :], 0.0)

        st = {'acc': None}

        def chunk(c):
            def f():
                if c == 0:
                    barrier(0)
                if c == WSPLIT:
                    barrier(1)
                if c == 0:
                    st['acc'] = acc_s[...] + b2s[...]
                st['acc'] = st['acc'] + ffn_chunk(xn2_s[...], c)
            return f
        tasks = ([functools.partial(halo, j) for j in (1, 2)]
                 + [functools.partial(shuffle_store, j, tmp.at[j], r0, SB) for j in range(3) for r0 in range(0, T, SB)]
                 + [functools.partial(ln_chain, functools.partial(load_x, u2), xn1, LB, LD, never)])
        interleave([chunk(c) for c in range(NC)], tasks, xn2_s, never, F0, NC - 1)
        xs[pl.ds(r, T), :] = st['acc']
        obuf[pl.ds(r, T), :] = st['acc'].astype(BF16)

        @pl.when(u >= NT)
        def _():
            out_copy(tile).start()
        return u
    last = lax.fori_loop(0, NU - 1, step, 0)

    def epi_wo(h):
        y = _dot(pltpu.bitcast(osc[h * TH // 2:(h + 1) * TH // 2, :], BF16), wo[...])
        x1 = xs[S - T + h * TH:S - T + (h + 1) * TH, :] + y
        xn2_s[h * TH:(h + 1) * TH, :] = _ln(x1).astype(BF16)
        acc_s[h * TH:(h + 1) * TH, :] = x1 + b2s[...]
        return y

    def epi_second(y0):
        if EG:
            attention(NT - 1, last < 0, TH // RB, T // RB, functools.partial(mm_clock, y0, RB), EG)
        else:
            attention(NT - 1, None, TH // RB, T // RB)
        epi_wo(1)

    attention(NT - 1, None, 0, TH // RB)
    y0 = epi_wo(0)
    if EPO:
        acc_s[0:TH, :] += ffn_chunk(xn2_s[0:TH, :], 0, lambda h: epi_second(jnp.concatenate([y0, h], axis=1)))
    else:
        epi_second(y0)
        acc_s[0:TH, :] += ffn_chunk(xn2_s[0:TH, :], 0)
    acc_s[TH:T, :] += ffn_chunk(xn2_s[TH:T, :], 0)

    def epi_body(c, carry):
        a = acc_s[...] + ffn_chunk(xn2_s[...], c)
        acc_s[...] = a
        obuf[S - T:S, :] = a.astype(BF16)
        return carry
    lax.fori_loop(1, NC, epi_body, 0)
    out_copy(NT - 1).start()
    for t in range(NT):
        out_copy(t).wait()


@jax.jit
def pallas_interleave_layers__sliding_local_dilated__dense_activation_gelu__prompt_kernel(
        A_x, A_wqkv, A_wo, B_x, B_w1, B_b1, B_w2, B_b2):
    B, S, D = A_x.shape
    F = B_w1.shape[1]
    G = D // 128
    NC = F // FC
    NT = S // T
    hbm = pl.BlockSpec(memory_space=pl.ANY)
    out = pl.pallas_call(
        kernel,
        in_specs=[hbm] * 7,
        out_specs=hbm,
        out_shape=jax.ShapeDtypeStruct((S, D), A_x.dtype),
        scratch_shapes=[pltpu.VMEM((3, D, D), BF16),
                        pltpu.VMEM((D, D), BF16),
                        pltpu.VMEM((D, F), BF16),
                        pltpu.VMEM((F, D), BF16),
                        pltpu.VMEM((S, D), BF16),
                        pltpu.VMEM((S, D), F32),
                        pltpu.VMEM((S, D), BF16),
                        pltpu.VMEM((3, G, T + HALO, 128), F32),
                        pltpu.VMEM((T, D), BF16),
                        pltpu.VMEM((T // 2, D), U32),
                        pltpu.VMEM((T, D), F32),
                        pltpu.VMEM((T, D), BF16),
                        pltpu.VMEM((3, T, D), F32),
                        pltpu.VMEM((NC, 1, FC), F32),
                        pltpu.VMEM((1, D), F32),
                        pltpu.VMEM((F,), BF16),
                        pltpu.VMEM((D,), BF16),
                        pltpu.SemaphoreType.DMA((4 + XS,)),
                        pltpu.SemaphoreType.DMA((9,)),
                        pltpu.SemaphoreType.DMA((4,)),
                        pltpu.SemaphoreType.DMA((NT,))],
        compiler_params=pltpu.CompilerParams(vmem_limit_bytes=100 * 1024 * 1024),
    )(A_x.reshape(S, D), A_wqkv, A_wo, B_w1, B_b1, B_w2, B_b2)
    return out.reshape(B, S, D)
```
